```python
import os as _os
_os.environ.setdefault('JAX_PLATFORMS', 'cpu')
import jax
import jax.numpy as jnp

def _softmax(x, axis=-1):
    return jax.nn.softmax(x, axis=axis)

def _gelu(x):
    return jax.nn.gelu(x, approximate=True)

def _silu(x):
    return jax.nn.silu(x)

def _sigmoid(x):
    return jax.nn.sigmoid(x)

def _layernorm(x, axis=-1, eps=1e-05):
    m = jnp.mean(x, axis=axis, keepdims=True)
    v = jnp.var(x, axis=axis, keepdims=True)
    return (x - m) / jnp.sqrt(v + eps)

def _scatter_add(tgt, idx, src, axis=0):
    return tgt.at[idx].add(src)

def _segment_sum(src, seg, n):
    return jax.ops.segment_sum(src, seg, n)

class _Rng:

    def __init__(self, key):
        self._k = key

    def _next(self):
        self._k, sub = jax.random.split(self._k)
        return sub

    def normal(self, shape):
        return jax.random.normal(self._next(), shape, dtype=jnp.bfloat16)

    def randint(self, lo, hi, shape):
        return jax.random.randint(self._next(), shape, lo, hi, dtype=jnp.int32)

    def uniform(self, shape, lo=0.0, hi=1.0):
        return jax.random.uniform(self._next(), shape, jnp.bfloat16, lo, hi)

    def permutation(self, n):
        return jax.random.permutation(self._next(), n)
kernel_name = 'sequential_preLN__linear_attn_block__mixer_gmlp__prompt'

def setup_inputs():
    _rng = _Rng(jax.random.key(int.from_bytes(__import__("os").urandom(4), "little")))
    _w = lambda a: (lambda t: t.astype(jnp.bfloat16) if jnp.issubdtype(t.dtype, jnp.floating) else t)(jnp.asarray(a))

    def _A_setup():
        B, S, D = (1, 2048, 512)
        return {'x': _w((lambda *s: _rng.normal(s) * 0.05)(B, S, D)), 'wqkv': _w((lambda *s: _rng.normal(s) * 0.05)(D, 3 * D)), 'wo': _w((lambda *s: _rng.normal(s) * 0.05)(D, D))}
    _A_in = _A_setup()

    def _B_setup():
        B, S, D, F = (1, 2048, 512, 1792)
        Fh = F // 2
        return {'x': _w((lambda *s: _rng.normal(s) * 0.05)(B, S, D)), 'w_in': _w((lambda *s: _rng.normal(s) * 0.4)(D, 2 * Fh)), 'w_sp': _w(0.01 * (lambda *s: _rng.normal(s) * 0.4)(S, S)), 'b_sp': _w(1.0 + 0.01 * (lambda *s: _rng.normal(s) * 0.05)(S)), 'w_out': _w((lambda *s: _rng.normal(s) * 0.05)(Fh, D))}
    _B_in = _B_setup()
    return {'A_x': _A_in['x'], 'A_wqkv': _A_in['wqkv'], 'A_wo': _A_in['wo'], 'B_x': _B_in['x'], 'B_w_in': _B_in['w_in'], 'B_w_sp': _B_in['w_sp'], 'B_b_sp': _B_in['b_sp'], 'B_w_out': _B_in['w_out']}

def reference(A_x, A_wqkv, A_wo, B_x, B_w_in, B_w_sp, B_b_sp, B_w_out):

    def _A_ref(x, wqkv, wo):
        B, S, D = x.shape
        H = 32
        Dh = D // H
        qkv = (lambda x, *d: x.transpose(*d))((x @ wqkv).reshape(B, S, 3, H, Dh), 2, 0, 3, 1, 4)
        q, k, v = (qkv[0], qkv[1], qkv[2])
        phi = lambda t: jnp.where(t > 0, t + 1, jnp.exp(t)) + 1e-06
        pq, pk = (phi(q), phi(k))
        kv = jnp.einsum('bhsd,bhse->bhde', pk, v)
        z = jnp.einsum('bhsd->bhd', pk)
        num = jnp.einsum('bhqd,bhde->bhqe', pq, kv)
        den = jnp.einsum('bhqd,bhd->bhq', pq, z)[..., None] + 1e-06
        o = num / den
        return (lambda x, *d: x.transpose(*d))(o, 0, 2, 1, 3).reshape(B, S, D) @ wo

    def _B_ref(x, w_in, w_sp, b_sp, w_out):
        B, S, D = x.shape
        F = w_in.shape[-1]
        Fh = F // 2
        z = _gelu(jnp.einsum('bsd,df->bsf', x, w_in))
        z1 = z[..., :Fh].copy()
        z2 = _layernorm(z[..., Fh:], axis=-1)
        g = jnp.einsum('ts,bsf->btf', w_sp, z2) + b_sp[None, :, None]
        return jnp.einsum('bsf,fd->bsd', z1 * g, w_out)
    x = A_x
    h = x + _A_ref(_layernorm(x, axis=-1), A_wqkv, A_wo)
    h2 = h + _B_ref(_layernorm(h, axis=-1), B_w_in, B_w_sp, B_b_sp, B_w_out)
    return h2
```

```python
import jax
import jax.numpy as jnp
import numpy as np
import jax.experimental.pallas as pl
import jax.experimental.pallas.tpu as pltpu

S, D, FH = 2048, 512, 896
TM1 = 256
TM2 = 256
TM3 = 256
F32 = jnp.float32
BF16 = jnp.bfloat16


def _ln(x, n):
    m = jnp.sum(x, axis=-1, keepdims=True) * (1.0 / n)
    xc = x - m
    v = jnp.sum(xc * xc, axis=-1, keepdims=True) * (1.0 / n)
    return xc * jax.lax.rsqrt(v + 1e-5)


def _phi(t):
    return jnp.where(t > 0, t + 1.0, jnp.exp(t)) + 1e-6


def _gelu(x):
    c = float(np.sqrt(2.0 / np.pi))
    inner = x * (c + (c * 0.044715) * (x * x))
    hx = 0.5 * x
    return hx * jnp.tanh(inner) + hx


def _dot(a, b):
    return jnp.dot(a, b, preferred_element_type=F32)


def kernel(x_hbm, wqkv_hbm, wo_hbm, win_hbm, wsp_hbm, bsp_hbm, wout_hbm, out_hbm,
           x_v, wqkv_v, wo_v, win_v, wsp_v, bsp_v, wout_v,
           xn_v, a_v, h_v, hn_v, z2_v, o_v, sems, osems):
    cps = [
        pltpu.make_async_copy(x_hbm, x_v, sems.at[0]),
        pltpu.make_async_copy(wqkv_hbm, wqkv_v, sems.at[1]),
        pltpu.make_async_copy(wo_hbm, wo_v, sems.at[2]),
        pltpu.make_async_copy(win_hbm, win_v, sems.at[3]),
        pltpu.make_async_copy(bsp_hbm, bsp_v, sems.at[4]),
        pltpu.make_async_copy(wout_hbm, wout_v, sems.at[5]),
        pltpu.make_async_copy(wsp_hbm, wsp_v, sems.at[6]),
    ]
    cps[0].start()
    cps[1].start()
    cps[0].wait()
    cps[1].wait()
    for c in cps[2:]:
        c.start()

    a_v[...] = jnp.zeros_like(a_v)

    def p1(i, zacc):
        r = pl.ds(pl.multiple_of(i * TM1, TM1), TM1)
        xn = _ln(x_v[r, :].astype(F32), D).astype(BF16)
        xn_v[r, :] = xn
        k = _dot(xn, wqkv_v[:, D:2 * D])
        pk = _phi(k).astype(BF16)
        a_v[...] += jax.lax.dot_general(pk, xn, (((0,), (0,)), ((), ())),
                                        preferred_element_type=F32)
        pkf = pk.astype(F32)
        return zacc + jnp.sum(pkf.reshape(TM1 // 8, 8, D), axis=0)

    zacc = jax.lax.fori_loop(0, S // TM1, p1, jnp.zeros((8, D), F32))
    z = jnp.sum(zacc, axis=0, keepdims=True)

    ri = jax.lax.broadcasted_iota(jnp.int32, (128, 128), 0) // 16
    ci = jax.lax.broadcasted_iota(jnp.int32, (128, 128), 1) // 16
    mask = ri == ci
    cps[2].wait()
    zb = []
    m_rows = []
    for b in range(4):
        sl = slice(128 * b, 128 * (b + 1))
        kv = _dot(a_v[sl, :].astype(BF16), wqkv_v[:, 2 * D + 128 * b:2 * D + 128 * (b + 1)])
        kv = jnp.where(mask, kv, 0.0).astype(BF16)
        m_rows.append(_dot(kv, wo_v[sl, :]).astype(BF16))
        zbt = jnp.where(mask, jnp.broadcast_to(z[:, sl], (128, 128)), 0.0)
        zb.append(zbt.T.astype(BF16))
    mo = jnp.concatenate(m_rows, axis=0)

    cps[3].wait()

    def p2(i, carry):
        r = pl.ds(pl.multiple_of(i * TM2, TM2), TM2)
        xn = xn_v[r, :]
        pq = _phi(_dot(xn, wqkv_v[:, 0:D])).astype(BF16)
        den = jnp.concatenate(
            [_dot(pq[:, 128 * b:128 * (b + 1)], zb[b]) for b in range(4)], axis=1) + 1e-6
        ps = (pq.astype(F32) / den).astype(BF16)
        h = x_v[r, :].astype(F32) + _dot(ps, mo)
        h_v[r, :] = h
        hn = _ln(h, D).astype(BF16)
        hn_v[r, :] = hn
        u2 = _gelu(_dot(hn, win_v[:, FH:]))
        z2_v[r, :] = _ln(u2, FH).astype(BF16)
        return carry

    jax.lax.fori_loop(0, S // TM2, p2, 0)

    cps[4].wait()
    cps[5].wait()
    cps[6].wait()

    bt = bsp_v[...].astype(F32).T

    ocps = []
    for i in range(S // TM3):
        r = slice(i * TM3, (i + 1) * TM3)
        z1 = _gelu(_dot(hn_v[r, :], win_v[:, :FH]))
        bcol = jnp.concatenate([bt[:, j:j + 1] for j in range(i * TM3 // 128, (i + 1) * TM3 // 128)], axis=0)
        g = _dot(wsp_v[r, :], z2_v[...]) + bcol
        o = _dot((z1 * g).astype(BF16), wout_v[...])
        o_v[r, :] = (h_v[r, :] + o).astype(BF16)
        c = pltpu.make_async_copy(o_v.at[r, :], out_hbm.at[r, :], osems.at[i])
        c.start()
        ocps.append(c)
    for c in ocps:
        c.wait()


@jax.jit
def pallas_sequential_preLN__linear_attn_block__mixer_gmlp__prompt_kernel(
    A_x, A_wqkv, A_wo, B_x, B_w_in, B_w_sp, B_b_sp, B_w_out,
):
    del B_x
    x = A_x.reshape(S, D)
    bsp = B_b_sp.reshape(16, 128)
    hbm = pl.BlockSpec(memory_space=pl.ANY)
    out = pl.pallas_call(
        kernel,
        in_specs=[hbm] * 7,
        out_specs=hbm,
        out_shape=jax.ShapeDtypeStruct((S, D), BF16),
        scratch_shapes=[
            pltpu.VMEM((S, D), BF16), pltpu.VMEM((D, 3 * D), BF16), pltpu.VMEM((D, D), BF16),
            pltpu.VMEM((D, 2 * FH), BF16), pltpu.VMEM((S, S), BF16), pltpu.VMEM((16, 128), BF16),
            pltpu.VMEM((FH, D), BF16),
            pltpu.VMEM((S, D), BF16), pltpu.VMEM((D, D), F32), pltpu.VMEM((S, D), F32),
            pltpu.VMEM((S, D), BF16), pltpu.VMEM((S, FH), BF16), pltpu.VMEM((S, D), BF16),
            pltpu.SemaphoreType.DMA((8,)), pltpu.SemaphoreType.DMA((S // TM3,)),
        ],
        compiler_params=pltpu.CompilerParams(vmem_limit_bytes=100 * 1024 * 1024),
    )(x, A_wqkv, A_wo, B_w_in, B_w_sp, bsp, B_w_out)
    return out.reshape(1, S, D)
```

```python
import jax
import jax.numpy as jnp
import numpy as np
import jax.experimental.pallas as pl
import jax.experimental.pallas.tpu as pltpu

S, D, FH = 2048, 512, 896
TM = 256
CH = 128
NT = S // TM
F32 = jnp.float32
BF16 = jnp.bfloat16


def _ln(x, n, eps=1e-5, post=1.0):
    m = jnp.sum(x, axis=-1, keepdims=True) * (1.0 / n)
    xc = x - m
    v = jnp.sum(xc * xc, axis=-1, keepdims=True) * (1.0 / n)
    r = jax.lax.rsqrt(v + eps)
    if post != 1.0:
        r = r * post
    return xc * r


def _phi(t):
    return jnp.where(t > 0, t + 1.0, jnp.exp(t)) + 1e-6


def _gelu(x):
    c = float(np.sqrt(2.0 / np.pi))
    inner = x * (c + (c * 0.044715) * (x * x))
    return x * jnp.tanh(inner) + x


def _dot(a, b):
    return jnp.dot(a, b, preferred_element_type=F32)


def kernel(x_hbm, wqkv_hbm, wo_hbm, win_hbm, wsp_hbm, bsp_hbm, wout_hbm, out_hbm,
           x_v, wqkv_v, wo_v, win_v, wsp_v, bsp_v, wout_v,
           h_v, hn_v, z2_v, o_v, sem):
    def rows(i):
        return slice(i * TM, (i + 1) * TM)

    def cp(src, dst, sem):
        return pltpu.make_async_copy(src, dst, sem)

    xc = [cp(x_hbm.at[rows(i), :], x_v.at[rows(i), :], sem.at[i]) for i in range(NT)]
    c_wq = cp(wqkv_hbm.at[:, 0:D], wqkv_v.at[:, 0:D], sem.at[8])
    c_wk = cp(wqkv_hbm.at[:, D:2 * D], wqkv_v.at[:, D:2 * D], sem.at[9])
    c_wv = cp(wqkv_hbm.at[:, 2 * D:], wqkv_v.at[:, 2 * D:], sem.at[10])
    c_wo = cp(wo_hbm, wo_v, sem.at[11])
    c_win2 = cp(win_hbm.at[:, FH:], win_v.at[:, FH:], sem.at[12])
    c_win1 = cp(win_hbm.at[:, :FH], win_v.at[:, :FH], sem.at[13])
    c_b = cp(bsp_hbm, bsp_v, sem.at[14])
    c_wout = cp(wout_hbm, wout_v, sem.at[15])
    sc = [cp(wsp_hbm.at[rows(i), :], wsp_v.at[rows(i), :], sem.at[16 + i]) for i in range(NT)]

    for c in [xc[0], c_wk] + xc[1:] + [c_wq, c_wv, c_wo, c_win2, c_win1, c_b, c_wout] + sc:
        c.start()

    ri = jax.lax.broadcasted_iota(jnp.int32, (128, 128), 0) // 16
    ci = jax.lax.broadcasted_iota(jnp.int32, (128, 128), 1) // 16
    mask = ri == ci

    st = {}

    def s_ln1(i):
        st['xn', i] = _ln(x_v[rows(i), :].astype(F32), D).astype(BF16)

    def s_k(i):
        pk = _phi(_dot(st['xn', i], wqkv_v[:, D:2 * D])).astype(BF16)
        st['pk', i] = pk
        zs = jnp.sum(pk.astype(F32).reshape(TM // 8, 8, D), axis=0)
        st['z'] = zs if i == 0 else st['z'] + zs

    def s_a(i):
        d = jax.lax.dot_general(st['pk', i], st['xn', i], (((0,), (0,)), ((), ())),
                                preferred_element_type=F32)
        st['a'] = d if i == 0 else st['a'] + d

    def s_mid1():
        z = jnp.sum(st['z'], axis=0, keepdims=True)
        a = st['a'].astype(BF16)
        st['zrow'] = z
        for b in range(4):
            sl = slice(128 * b, 128 * (b + 1))
            kv = _dot(a[sl, :], wqkv_v[:, 2 * D + 128 * b:2 * D + 128 * (b + 1)])
            st['kv', b] = jnp.where(mask, kv, 0.0).astype(BF16)

    def s_mid2():
        st['mo'] = jnp.concatenate(
            [_dot(st['kv', b], wo_v[128 * b:128 * (b + 1), :]).astype(BF16) for b in range(4)], axis=0)

    def s_q(i):
        st['pq', i] = _phi(_dot(st['xn', i], wqkv_v[:, 0:D]))

    def s_den(i):
        pq = st['pq', i]
        z = st['zrow']
        lane = jax.lax.broadcasted_iota(jnp.int32, (TM, 128), 1)
        b8 = (lane & 8) == 0
        b4 = (lane & 4) == 0
        b3 = (lane & 3) == 0

        def rl(x, sh):
            return pltpu.roll(x, sh % 128, 1)

        q4 = [pq[:, 128 * b:128 * (b + 1)] for b in range(4)]
        p = [q4[b] * z[:, 128 * b:128 * (b + 1)] for b in range(4)]
        ab = jnp.where(b8, p[0] + rl(p[0], -8), p[1] + rl(p[1], 8))
        cd = jnp.where(b8, p[2] + rl(p[2], -8), p[3] + rl(p[3], 8))
        x = jnp.where(b4, ab + rl(ab, -4), cd + rl(cd, 4))
        y = x + rl(x, -2)
        y = y + rl(y, -1)
        r = jnp.where(b3, pl.reciprocal(y + 1e-6, approx=True), 0.0)
        r = r + rl(r, 1)
        r = r + rl(r, 2)
        rab = jnp.where(b4, r, rl(r, 4))
        rcd = jnp.where(b4, rl(r, -4), r)
        rr = [jnp.where(b8, rab, rl(rab, 8)), jnp.where(b8, rl(rab, -8), rab),
              jnp.where(b8, rcd, rl(rcd, 8)), jnp.where(b8, rl(rcd, -8), rcd)]
        st['ps', i] = jnp.concatenate([q4[b] * rr[b] for b in range(4)], axis=1).astype(BF16)

    def s_o(i):
        o = _dot(st['ps', i], st['mo'])
        for c in range(TM // CH):
            rr = slice(i * TM + c * CH, i * TM + (c + 1) * CH)
            h = x_v[rr, :].astype(F32) + o[c * CH:(c + 1) * CH]
            h_v[rr, :] = h
            hn_v[rr, :] = _ln(h, D).astype(BF16)

    def s_u2(i):
        u = _dot(hn_v[rows(i), :], win_v[:, FH:])
        zs = []
        for c in range(TM // CH):
            rr = slice(i * TM + c * CH, i * TM + (c + 1) * CH)
            z2 = _ln(_gelu(u[c * CH:(c + 1) * CH]), FH, 4e-5, 0.5).astype(BF16)
            zs.append(z2)
        st['z2', i] = jnp.concatenate(zs, axis=0)

    def s_z1(i):
        st['z1', i] = _gelu(_dot(hn_v[rows(i), :], win_v[:, :FH]))

    def s_g0(t):
        d = _dot(wsp_v[rows(0), rows(t)], st['z2', t])
        st['g0'] = d if t == 0 else st['g0'] + d
        z2_v[rows(t), :] = st['z2', t]

    def s_g(i):
        bcol = jnp.concatenate([st['bt'][:, j:j + 1] for j in range(i * TM // 128, (i + 1) * TM // 128)], axis=0)
        g = (st['g0'] if i == 0 else _dot(wsp_v[rows(i), :], z2_v[...])) + bcol
        st['zg', i] = (st['z1', i] * g).astype(BF16)

    ocps = []

    def s_out(i):
        nsplit = 2 if i == NT - 1 else 1
        hm = TM // nsplit
        for j in range(nsplit):
            rr = slice(i * TM + j * hm, i * TM + (j + 1) * hm)
            o = _dot(st['zg', i][j * hm:(j + 1) * hm], wout_v[...])
            o_v[rr, :] = (h_v[rr, :] + o).astype(BF16)
            c = cp(o_v.at[rr, :], out_hbm.at[rr, :], sem.at[24 + i + j])
            c.start()
            ocps.append(c)

    xc[0].wait()
    s_ln1(0)
    c_wk.wait()
    xc[1].wait()
    s_k(0)
    s_ln1(1)
    xc[2].wait()
    xc[3].wait()
    s_k(1)
    s_ln1(2)
    s_a(0)
    s_ln1(3)
    s_k(2)
    for c in xc[4:]:
        c.wait()
    s_a(1)
    for i in range(3, NT):
        s_k(i)
        if i + 1 < NT:
            s_ln1(i + 1)
        s_a(i - 1)
    for c in [c_wq, c_wv, c_wo, c_win2, c_win1, c_b, c_wout, sc[0]]:
        c.wait()
    s_q(0)
    s_a(NT - 1)
    s_q(1)
    s_mid1()
    s_q(2)
    s_mid2()
    st['bt'] = (0.5 * bsp_v[...].astype(F32)).T
    s_den(0)
    s_den(1)
    s_den(2)
    s_o(0)
    s_o(1)
    for t in range(NT):
        s_u2(t)
        if t + 3 < NT:
            s_q(t + 3)
            s_den(t + 3)
        if t >= 1:
            s_g0(t - 1)
        if t + 2 < NT:
            s_o(t + 2)
    s_z1(0)
    s_g0(NT - 1)
    for c in sc[1:]:
        c.wait()
    for i in range(NT):
        if i + 1 < NT:
            s_z1(i + 1)
        s_g(i)
        s_out(i)
    for c in ocps:
        c.wait()


@jax.jit
def pallas_sequential_preLN__linear_attn_block__mixer_gmlp__prompt_kernel(
    A_x, A_wqkv, A_wo, B_x, B_w_in, B_w_sp, B_b_sp, B_w_out,
):
    del B_x
    x = A_x.reshape(S, D)
    bsp = B_b_sp.reshape(16, 128)
    hbm = pl.BlockSpec(memory_space=pl.ANY)
    out = pl.pallas_call(
        kernel,
        in_specs=[hbm] * 7,
        out_specs=hbm,
        out_shape=jax.ShapeDtypeStruct((S, D), BF16),
        scratch_shapes=[
            pltpu.VMEM((S, D), BF16), pltpu.VMEM((D, 3 * D), BF16), pltpu.VMEM((D, D), BF16),
            pltpu.VMEM((D, 2 * FH), BF16), pltpu.VMEM((S, S), BF16), pltpu.VMEM((16, 128), BF16),
            pltpu.VMEM((FH, D), BF16),
            pltpu.VMEM((S, D), F32),
            pltpu.VMEM((S, D), BF16), pltpu.VMEM((S, FH), BF16), pltpu.VMEM((S, D), BF16),
            pltpu.SemaphoreType.DMA((34,)),
        ],
        compiler_params=pltpu.CompilerParams(vmem_limit_bytes=100 * 1024 * 1024, flags={'XLA_TPU_FORCE_LP_LLO_SCHEDULER': True}),
    )(x, A_wqkv, A_wo, B_w_in, B_w_sp, bsp, B_w_out)
    return out.reshape(1, S, D)
```
